```python
import jax
import jax.numpy as jnp

def _softmax(x, axis=-1):
    return jax.nn.softmax(x, axis=axis)
def _gelu(x):
    return jax.nn.gelu(x, approximate=True)
def _silu(x):
    return jax.nn.silu(x)
def _sigmoid(x):
    return jax.nn.sigmoid(x)
def _layernorm(x, axis=-1, eps=1e-5):
    m = jnp.mean(x, axis=axis, keepdims=True)
    v = jnp.var(x, axis=axis, keepdims=True)
    return (x - m) / jnp.sqrt(v + eps)
def _scatter_add(tgt, idx, src, axis=0):
    return tgt.at[idx].add(src)
def _segment_sum(src, seg, n):
    return jax.ops.segment_sum(src, seg, n)
class _Rng:
    def __init__(self, key):
        self._k = key
    def _next(self):
        self._k, sub = jax.random.split(self._k)
        return sub
    def normal(self, shape):
        return jax.random.normal(self._next(), shape, dtype=jnp.bfloat16)
    def randint(self, lo, hi, shape):
        return jax.random.randint(self._next(), shape, lo, hi, dtype=jnp.int32)
    def uniform(self, shape, lo=0.0, hi=1.0):
        return jax.random.uniform(self._next(), shape, jnp.bfloat16, lo, hi)
    def permutation(self, n):
        return jax.random.permutation(self._next(), n)


kernel_name = 'standalone__layernorm_linear__prompt'

def setup_inputs():
    _rng = _Rng(jax.random.key(int.from_bytes(__import__("os").urandom(4), "little")))
    _w = (lambda a: (lambda t: t.astype(jnp.bfloat16) if jnp.issubdtype(t.dtype, jnp.floating) else t)(jnp.asarray(a)))
    B, S, D = 2, 2048, 1024
    return {
        "x": _w((lambda *s: _rng.normal(s) * 0.05)(B, S, D)),
        "g": _w((lambda *s: _rng.normal(s) * 0.05)(D) + 1.0),
        "b": _w((lambda *s: _rng.normal(s) * 0.05)(D)),
        "w": _w((lambda *s: _rng.normal(s) * 0.05)(D, D)),
    }

def reference(x, g, b, w):
    return (_layernorm(x, axis=-1) * g + b) @ w
```

```python
import functools
import jax
import jax.numpy as jnp
import jax.experimental.pallas as pl
import jax.experimental.pallas.tpu as pltpu

M, D, N = 4096, 1024, 1024

def ln(x, g, b):
    x = x.astype(jnp.float32)
    m = jnp.sum(x, axis=-1, keepdims=True) * (1.0 / x.shape[-1])
    xc = x - m
    v = jnp.sum(xc * xc, axis=-1, keepdims=True) * (1.0 / x.shape[-1])
    rs = jax.lax.rsqrt(v + 1e-5)
    y = xc * rs
    y = y * g + b
    return y.astype(jnp.bfloat16), rs

def make_v8(R=128, xgroups=(2, 1, 5, 8, 16), wpieces=(2, 2, 2, 2), dma_order=None, nfirst=2,
            tail_split=4, flags=None, vmem=100*1024*1024, barrier_starts=True, ogroup=1, **cp):
    nc = M // R
    assert sum(xgroups) == nc and sum(wpieces) == 8
    gstart = [sum(xgroups[:i]) for i in range(len(xgroups))]
    wstart = [sum(wpieces[:i]) for i in range(len(wpieces))]
    chunk_group = []
    for gi, n in enumerate(xgroups):
        chunk_group += [gi] * n
    NP = 8
    r = R // NP
    if dma_order is None:
        dma_order = ["x0", "g", "b"] + [f"w{j}" for j in range(len(wpieces))] + [f"x{i}" for i in range(1, len(xgroups))]

    def kern(x_hbm, g_hbm, b_hbm, w_hbm, o_hbm, xbuf, gbuf, bbuf, wbuf, xsem, gsem, wsem, osem, rsem, *obufs):
        def xcopy(i):
            return pltpu.make_async_copy(x_hbm.at[pl.ds(gstart[i]*R, xgroups[i]*R), :], xbuf.at[pl.ds(gstart[i]*R, xgroups[i]*R), :], xsem.at[i])
        def wcopy(j):
            return pltpu.make_async_copy(w_hbm.at[:, pl.ds(wstart[j]*128, wpieces[j]*128)], wbuf.at[:, pl.ds(wstart[j]*128, wpieces[j]*128)], wsem.at[j])
        gc = pltpu.make_async_copy(g_hbm, gbuf, gsem.at[0])
        bc = pltpu.make_async_copy(b_hbm, bbuf, gsem.at[1])
        def get(name):
            if name == "g": return gc
            if name == "b": return bc
            if name[0] == "x": return xcopy(int(name[1:]))
            return wcopy(int(name[1:]))
        for i, name in enumerate(dma_order):
            get(name).start()
            if barrier_starts and name not in ("g", "b"):
                pl.semaphore_signal(rsem, 1)
                pl.semaphore_wait(rsem, 1)
        waited = set()
        def wait(name):
            if name not in waited:
                waited.add(name)
                get(name).wait()
        ocopies = []
        def ostart(c, c0, c1):
            cp_ = pltpu.make_async_copy(obufs[c].at[:, pl.ds(c0, c1 - c0)], o_hbm.at[pl.ds(c*R, R), pl.ds(c0, c1 - c0)], osem)
            cp_.start()
            ocopies.append(cp_)

        wait("g"); wait("b")
        g2 = gbuf[...].astype(jnp.float32)
        b2 = bbuf[...].astype(jnp.float32)
        g = jnp.concatenate([g2[q:q+1, :] for q in range(8)], axis=1)
        b = jnp.concatenate([b2[q:q+1, :] for q in range(8)], axis=1)

        def lnp(c, p):
            y, rs = ln(xbuf[c*R + p*r: c*R + (p+1)*r, :], g, b)
            yu = pltpu.bitcast(y, jnp.uint32)
            t = rs[0:8]
            for rr in range(1, r // 8):
                t = jnp.minimum(t, rs[rr*8:(rr+1)*8])
            mask = jnp.broadcast_to(t, (8, 128)) < -1.0
            return yu, mask
        def tied(yu, masks):
            tl = yu[0:8, 0:128]
            for mk in masks:
                tl = jnp.where(mk, jnp.uint32(0), tl)
            top = jnp.concatenate([tl, yu[0:8, 128:]], axis=1)
            return jnp.concatenate([top, yu[8:, :]], axis=0)
        def dot(c, yu, n0, n1, masks):
            yy = tied(yu, masks) if masks else yu
            obufs[c][:, n0*128:n1*128] = jnp.dot(pltpu.bitcast(yy, jnp.bfloat16), wbuf[:, n0*128:n1*128],
                                                 preferred_element_type=jnp.float32).astype(o_hbm.dtype)

        ys = {}
        for c in range(nfirst):
            wait(f"x{chunk_group[c]}")
            ys[c] = jnp.concatenate([lnp(c, p)[0] for p in range(NP)], axis=0)
        slots = []
        for j in range(len(wpieces)):
            for c in range(nfirst):
                for n in range(wstart[j], wstart[j] + wpieces[j]):
                    slots.append((j, c, n))
        nxt_c = nfirst
        tie_slots = slots[-(NP):]
        lastpiece_first = min(i for i, s in enumerate(slots) if s[0] == len(wpieces) - 1)
        xw_at = max(0, len(slots) - NP)
        bidx = [i for i, s in enumerate(slots) if i == 0 or slots[i-1][0] != s[0]]
        xw_at = max(i for i in bidx if i <= xw_at)
        avail = list(range(xw_at + 1, len(slots)))
        nxt = {}
        tie_map = {}
        for q in range(NP - 1):
            pos = avail[min(len(avail) - 1, (q * len(avail)) // (NP - 1))]
            tie_map.setdefault(pos, []).append(q)
        for i, (j, c, n) in enumerate(slots):
            if i in bidx:
                wait(f"w{j}")
            if i == xw_at:
                wait(f"x{chunk_group[nxt_c]}")
                for q in range(NP):
                    nxt[q] = lnp(nxt_c, q)
            masks = [nxt[q][1] for q in tie_map.get(i, [])]
            dot(c, ys[c], n, n + 1, masks)
            if n == 7:
                ostart(c, 0, N)
        cur = jnp.concatenate([nxt[q][0] for q in range(NP)], axis=0)
        for c in range(nfirst, nc):
            nxt = {}
            if c + 1 < nc:
                wait(f"x{chunk_group[c+1]}")
                for q in range(NP):
                    nxt[q] = lnp(c + 1, q)
            for n in range(8):
                masks = [nxt[n - 1][1]] if (c + 1 < nc and n >= 1) else []
                dot(c, cur, n, n + 1, masks)
                if c == nc - 1 and tail_split > 1:
                    w_ = 8 // tail_split
                    if (n + 1) % w_ == 0:
                        ostart(c, (n + 1 - w_) * 128, (n + 1) * 128)
            if not (c == nc - 1 and tail_split > 1):
                ostart(c, 0, N)
            if c + 1 < nc:
                cur = jnp.concatenate([nxt[q][0] for q in range(NP)], axis=0)
        for cp_ in ocopies:
            cp_.wait()

    def fn(x, g, b, w):
        B, S, _ = x.shape
        x2 = x.reshape(M, D)
        anyspec = pl.BlockSpec(memory_space=pl.ANY)
        out = pl.pallas_call(
            kern,
            in_specs=[anyspec] * 4,
            out_specs=anyspec,
            out_shape=jax.ShapeDtypeStruct((M, N), x.dtype),
            scratch_shapes=[
                pltpu.VMEM((M, D), jnp.bfloat16),
                pltpu.VMEM((8, 128), jnp.bfloat16),
                pltpu.VMEM((8, 128), jnp.bfloat16),
                pltpu.VMEM((D, N), jnp.bfloat16),
                pltpu.SemaphoreType.DMA((len(xgroups),)),
                pltpu.SemaphoreType.DMA((2,)),
                pltpu.SemaphoreType.DMA((len(wpieces),)),
                pltpu.SemaphoreType.DMA(()),
                pltpu.SemaphoreType.REGULAR(()),
            ] + [pltpu.VMEM((R, N), jnp.bfloat16) for c in range(nc)],
            compiler_params=pltpu.CompilerParams(vmem_limit_bytes=vmem, flags=flags, disable_semaphore_checks=True, **cp),
        )(x2, g.reshape(8, 128), b.reshape(8, 128), w)
        return out.reshape(B, S, N)
    return fn


_fn = make_v8(tail_split=8)


@jax.jit
def pallas_standalone__layernorm_linear__prompt_kernel(x, g, b, w):
    return _fn(x, g, b, w)
```

```python
import functools
import jax
import jax.numpy as jnp
import jax.experimental.pallas as pl
import jax.experimental.pallas.tpu as pltpu

M, D, N = 4096, 1024, 1024
H = 512

def ln_f32(x, g, b):
    x = x.astype(jnp.float32)
    m = jnp.sum(x, axis=-1, keepdims=True) * (1.0 / x.shape[-1])
    xc = x - m
    v = jnp.sum(xc * xc, axis=-1, keepdims=True) * (1.0 / x.shape[-1])
    rs = jax.lax.rsqrt(v + 1e-5)
    y = xc * rs
    y = y * g + b
    return y, rs

def make_s8(R=64, F=2, xgroups=(2, 2, 4, 8, 16), dma_order=None, tail_split=True, oprio=0,
            perm=(1, 4, 3, 2, 0, 5, 6), flags=None, vmem=100*1024*1024, xw_j=2, olate=False, tpos=(6,13,20), tpos1=None, tiek=(0,), nowait=False, **cp):
    nb = M // (2 * R)
    assert sum(xgroups) == nb
    gstart = [sum(xgroups[:i]) for i in range(len(xgroups))]
    blk_group = []
    for gi, n in enumerate(xgroups):
        blk_group += [gi] * n
    NQ = R // 16
    BR = 2 * R
    if dma_order is None:
        dma_order = ["x0", "g", "b", "w0", "w1", "x1", "w2", "w3"] + [f"x{i}" for i in range(2, len(xgroups))]

    def kern(x_hbm, g_hbm, b_hbm, w_hbm, o_hbm, xbuf, gbuf, bbuf, wbuf, bsc, xsem, gsem, wsem, osem, rsem, *obufs):
        def copies(name):
            if name == "g": return [pltpu.make_async_copy(g_hbm, gbuf, gsem.at[0])]
            if name == "b": return [pltpu.make_async_copy(b_hbm, bbuf, gsem.at[1])]
            i = int(name[1:])
            if name[0] == "x":
                sl = pl.ds(gstart[i]*BR, xgroups[i]*BR)
                return [pltpu.make_async_copy(x_hbm.at[sl, :], xbuf.at[sl, :], xsem.at[i])]
            return [pltpu.make_async_copy(w_hbm.at[:, pl.ds(c0 + i*128, 128)], wbuf.at[:, pl.ds(c0 + i*128, 128)], wsem.at[2*i + h])
                    for h, c0 in enumerate((0, H))]
        for name in dma_order:
            for c in copies(name):
                c.start()
            if name not in ("g", "b"):
                pl.semaphore_signal(rsem, 1)
                pl.semaphore_wait(rsem, 1)
        waited = set()
        def wait(name):
            if name not in waited:
                waited.add(name)
                for c in copies(name):
                    c.wait()
        ocopies = []
        def ostart(blk, r0, r1, c0, c1):
            cp_ = pltpu.make_async_copy(obufs[blk].at[pl.ds(r0, r1 - r0), pl.ds(c0, c1 - c0)],
                                        o_hbm.at[pl.ds(blk*BR + r0, r1 - r0), pl.ds(c0, c1 - c0)], osem)
            cp_.start(priority=oprio)
            ocopies.append(cp_)

        wait("g"); wait("b")
        g2 = gbuf[...].astype(jnp.float32)
        b2 = bbuf[...].astype(jnp.float32)
        g = jnp.concatenate([g2[q:q+1, :] for q in range(8)], axis=1)
        b = jnp.concatenate([b2[q:q+1, :] for q in range(8)], axis=1)

        def lnp(blk, q):
            r0 = blk * BR + q * 16
            yt, rt = ln_f32(xbuf[r0:r0+16, :], g, b)
            yb, rb = ln_f32(xbuf[r0+R:r0+R+16, :], g, b)
            a11, a12, a21, a22 = yt[:, :H], yt[:, H:], yb[:, :H], yb[:, H:]
            ops = [a11 + a22, a21 + a22, a11, a22, a11 + a12, a21 - a11, a12 - a22]
            ops = [pltpu.bitcast(o.astype(jnp.bfloat16), jnp.uint32) for o in ops]
            t = jnp.minimum(jnp.minimum(rt[0:8], rt[8:16]), jnp.minimum(rb[0:8], rb[8:16]))
            mask = jnp.broadcast_to(t, (8, 128)) < -1.0
            return ops, mask
        def tied(yu, masks):
            parts = []
            for c in range(4):
                tl = yu[0:8, c*128:(c+1)*128]
                if c in tiek:
                    for mk in masks:
                        tl = jnp.where(mk, jnp.uint32(0), tl)
                parts.append(tl)
            top = jnp.concatenate(parts, axis=1)
            return jnp.concatenate([top, yu[8:, :]], axis=0)
        def bops(j):
            b11 = wbuf[0:H, j*128:(j+1)*128]
            b21 = wbuf[H:2*H, j*128:(j+1)*128]
            b12 = wbuf[0:H, H+j*128:H+(j+1)*128]
            b22 = wbuf[H:2*H, H+j*128:H+(j+1)*128]
            f = lambda a: a.astype(jnp.float32)
            c = lambda a: a.astype(jnp.bfloat16)
            ops = [c(f(b11) + f(b22)), b11, c(f(b12) - f(b22)), c(f(b21) - f(b11)), b22, c(f(b11) + f(b12)), c(f(b21) + f(b22))]
            for i in range(7):
                bsc[j * 7 + i] = pltpu.bitcast(ops[i], jnp.uint32)
            return None
        def products(blk, A, Bj, j, tie_fn):
            Ms = {}
            for s, i in enumerate(perm):
                masks = tie_fn(s)
                a = tied(A[i], masks) if masks else A[i]
                Ms[i] = jnp.dot(pltpu.bitcast(a, jnp.bfloat16), pltpu.bitcast(bsc[j * 7 + i], jnp.bfloat16), preferred_element_type=jnp.float32)
            ob = obufs[blk]
            dt = ob.dtype
            ob[0:R, j*128:(j+1)*128] = (Ms[0] + Ms[3] - Ms[4] + Ms[6]).astype(dt)
            ob[0:R, H+j*128:H+(j+1)*128] = (Ms[2] + Ms[4]).astype(dt)
            ob[R:BR, j*128:(j+1)*128] = (Ms[1] + Ms[3]).astype(dt)
            ob[R:BR, H+j*128:H+(j+1)*128] = (Ms[0] - Ms[1] + Ms[2] + Ms[5]).astype(dt)
        def catA(pieces):
            return [jnp.concatenate([pieces[q][0][i] for q in range(NQ)], axis=0) for i in range(7)]

        As = []
        for blk in range(F):
            wait(f"x{blk_group[blk]}")
            As.append(catA([lnp(blk, q) for q in range(NQ)]))
        Bs = []
        nxt = None
        nslots_after = (4 - xw_j) * F * 7
        for j in range(4):
            wait(f"w{j}")
            if j == xw_j:
                wait(f"x{blk_group[F]}")
                nxt = [lnp(F, q) for q in range(NQ)]
            Bs.append(bops(j))
            for blk in range(F):
                base = ((j - xw_j) * F + blk) * 7
                def tie_fn(s, base=base):
                    if nxt is None or base < 0: return []
                    slot = base + s
                    return [nxt[q][1] for q in range(NQ - 1) if (tpos1[q] if tpos1 else 6 + (q * (nslots_after - 8)) // (NQ - 1)) == slot]
                products(blk, As[blk], Bs[j], j, tie_fn)
        for blk in range(F):
            ostart(blk, 0, BR, 0, N)
        cur = nxt
        for blk in range(F, nb):
            A = catA(cur)
            nxt = None
            if blk + 1 < nb:
                wait(f"x{blk_group[blk+1]}")
                nxt = [lnp(blk + 1, q) for q in range(NQ)]
            for j in range(4):
                def tie_fn(s, j=j):
                    if nxt is None: return []
                    slot = j * 7 + s
                    return [nxt[q if NQ - 1 == len(tpos) else 0][1] for q in range(len(tpos)) if tpos[q] == slot]
                products(blk, A, Bs[j], j, tie_fn)
                if blk == nb - 1 and tail_split:
                    ostart(blk, 0, BR, j*128, (j+1)*128)
                    ostart(blk, 0, BR, H+j*128, H+(j+1)*128)
            if not (blk == nb - 1 and tail_split) and not olate:
                ostart(blk, 0, BR, 0, N)
            cur = nxt
        if olate:
            for blk in range(F, nb - 1):
                ostart(blk, 0, BR, 0, N)
        for cp_ in ocopies:
            cp_.wait()

    def fn(x, g, b, w):
        B, S, _ = x.shape
        x2 = x.reshape(M, D)
        anyspec = pl.BlockSpec(memory_space=pl.ANY)
        out = pl.pallas_call(
            kern,
            in_specs=[anyspec] * 4,
            out_specs=anyspec,
            out_shape=jax.ShapeDtypeStruct((M, N), x.dtype),
            scratch_shapes=[
                pltpu.VMEM((M, D), jnp.bfloat16),
                pltpu.VMEM((8, 128), jnp.bfloat16),
                pltpu.VMEM((8, 128), jnp.bfloat16),
                pltpu.VMEM((D, N), jnp.bfloat16),
                pltpu.VMEM((28, 256, 128), jnp.uint32),
                pltpu.SemaphoreType.DMA((len(xgroups),)),
                pltpu.SemaphoreType.DMA((2,)),
                pltpu.SemaphoreType.DMA((8,)),
                pltpu.SemaphoreType.DMA(()),
                pltpu.SemaphoreType.REGULAR(()),
            ] + [pltpu.VMEM((BR, N), jnp.bfloat16) for c in range(nb)],
            compiler_params=pltpu.CompilerParams(vmem_limit_bytes=vmem, flags=flags, disable_semaphore_checks=True, **cp),
        )(x2, g.reshape(8, 128), b.reshape(8, 128), w)
        return out.reshape(B, S, N)
    return fn


_fn = make_s8(tiek=(0, 1, 2, 3), tpos=(5, 10, 15))


@jax.jit
def pallas_standalone__layernorm_linear__prompt_kernel(x, g, b, w):
    return _fn(x, g, b, w)
```

```python
import jax
import jax.numpy as jnp
import jax.experimental.pallas as pl
import jax.experimental.pallas.tpu as pltpu

_EPS = 1e-5
_R = 64
_BR = 2 * _R
_NQ = _R // 16
_PERM = (1, 3, 4, 2, 0, 5, 6)
_TIE_SLOTS = (7, 14, 21)
_X_GROUPS = (2, 1, 2, 8, 19)
_DMA_ORDER = ("g", "b", "x0", "w0", "w1", "w2", "x1", "w3", "x2", "x3", "x4")
_STARTUP = (
    (("g", "b", "x0"), (0, 1), ()),
    (("w0",), (), ((0, 0), (1, 0))),
    (("w1",), (), ((0, 1), (1, 1))),
    (("w2", "x1"), (2,), ((0, 2), (1, 2), (2, 0), (2, 1), (2, 2))),
    (("w3", "x2"), (3,), ((0, 3), (1, 3), (2, 3))),
)
_N_STARTUP = 3


def _layernorm(x, g, b):
    x = x.astype(jnp.float32)
    inv_d = 1.0 / x.shape[-1]
    m = jnp.sum(x, axis=-1, keepdims=True) * inv_d
    xc = x - m
    v = jnp.sum(xc * xc, axis=-1, keepdims=True) * inv_d
    rstd = jax.lax.rsqrt(v + _EPS)
    return xc * rstd * g + b, rstd


def _make_kernel(M, D, N):
    assert D == N == 1024 and M % _BR == 0 and sum(_X_GROUPS) == M // _BR
    H = D // 2
    nb = M // _BR
    gstart = [sum(_X_GROUPS[:i]) for i in range(len(_X_GROUPS))]
    blk_group = [gi for gi, n in enumerate(_X_GROUPS) for _ in range(n)]

    def kernel(x_hbm, g_hbm, b_hbm, w_hbm, o_hbm,
               xbuf, gbuf, bbuf, wbuf, xsem, gsem, wsem, osem, rsem, *obufs):
        def copies(name):
            if name == "g":
                return [pltpu.make_async_copy(g_hbm, gbuf, gsem.at[0])]
            if name == "b":
                return [pltpu.make_async_copy(b_hbm, bbuf, gsem.at[1])]
            i = int(name[1:])
            if name[0] == "x":
                rows = pl.ds(gstart[i] * _BR, _X_GROUPS[i] * _BR)
                return [pltpu.make_async_copy(x_hbm.at[rows, :], xbuf.at[rows, :], xsem.at[i])]
            return [
                pltpu.make_async_copy(
                    w_hbm.at[:, pl.ds(c0 + i * 128, 128)],
                    wbuf.at[:, pl.ds(c0 + i * 128, 128)],
                    wsem.at[2 * i + h])
                for h, c0 in enumerate((0, H))
            ]

        for name in _DMA_ORDER:
            for c in copies(name):
                c.start()
            if name != "g":
                pl.semaphore_signal(rsem, 1)
                pl.semaphore_wait(rsem, 1)

        waited = set()

        def wait(name):
            if name not in waited:
                waited.add(name)
                for c in copies(name):
                    c.wait()

        out_copies = []
        held_back = []
        released = [False]

        def out_start(blk, c0, c1):
            if not released[0]:
                held_back.append((blk, c0, c1))
                return
            cp = pltpu.make_async_copy(
                obufs[blk].at[:, pl.ds(c0, c1 - c0)],
                o_hbm.at[pl.ds(blk * _BR, _BR), pl.ds(c0, c1 - c0)],
                osem)
            cp.start()
            out_copies.append(cp)

        def release_outputs():
            released[0] = True
            for args in held_back:
                out_start(*args)

        gb = []

        def get_gb():
            if not gb:
                g2 = gbuf[...].astype(jnp.float32)
                b2 = bbuf[...].astype(jnp.float32)
                gb.append(jnp.concatenate([g2[q:q + 1, :] for q in range(8)], axis=1))
                gb.append(jnp.concatenate([b2[q:q + 1, :] for q in range(8)], axis=1))
            return gb

        def ln_piece(blk, q):
            g, b = get_gb()
            r0 = blk * _BR + q * 16
            yt, rt = _layernorm(xbuf[r0:r0 + 16, :], g, b)
            yb, rb = _layernorm(xbuf[r0 + _R:r0 + _R + 16, :], g, b)
            a11, a12, a21, a22 = yt[:, :H], yt[:, H:], yb[:, :H], yb[:, H:]
            ops = [a11 + a22, a21 + a22, a11, a22, a11 + a12, a21 - a11, a12 - a22]
            ops = [pltpu.bitcast(o.astype(jnp.bfloat16), jnp.uint32) for o in ops]
            t = jnp.minimum(jnp.minimum(rt[0:8], rt[8:16]), jnp.minimum(rb[0:8], rb[8:16]))
            never = jnp.broadcast_to(t, (8, 128)) < -1.0
            return ops, never

        def left_operands(pieces):
            return [jnp.concatenate([p[0][i] for p in pieces], axis=0) for i in range(7)]

        def tie(a, masks):
            parts = []
            for c in range(4):
                t = a[0:8, c * 128:(c + 1) * 128]
                for mk in masks:
                    t = jnp.where(mk, jnp.uint32(0), t)
                parts.append(t)
            return jnp.concatenate([jnp.concatenate(parts, axis=1), a[8:, :]], axis=0)

        right = {}

        def right_operand(j, i):
            if j not in right:
                b11 = wbuf[0:H, j * 128:(j + 1) * 128]
                b21 = wbuf[H:D, j * 128:(j + 1) * 128]
                b12 = wbuf[0:H, H + j * 128:H + (j + 1) * 128]
                b22 = wbuf[H:D, H + j * 128:H + (j + 1) * 128]
                f = lambda a: a.astype(jnp.float32)
                c = lambda a: a.astype(jnp.bfloat16)
                right[j] = [c(f(b11) + f(b22)), b11, c(f(b12) - f(b22)), c(f(b21) - f(b11)),
                            b22, c(f(b11) + f(b12)), c(f(b21) + f(b22))]
            return right[j][i]

        def combine(blk, j, m):
            ob = obufs[blk]
            dt = ob.dtype
            lo, hi = j * 128, H + j * 128
            ob[0:_R, lo:lo + 128] = (m[0] + m[3] - m[4] + m[6]).astype(dt)
            ob[0:_R, hi:hi + 128] = (m[2] + m[4]).astype(dt)
            ob[_R:_BR, lo:lo + 128] = (m[1] + m[3]).astype(dt)
            ob[_R:_BR, hi:hi + 128] = (m[0] - m[1] + m[2] + m[5]).astype(dt)

        def products(a_ops, j, masks_for_slot):
            m = {}
            for s, i in enumerate(_PERM):
                masks = masks_for_slot(s)
                a = tie(a_ops[i], masks) if masks else a_ops[i]
                m[i] = jnp.dot(pltpu.bitcast(a, jnp.bfloat16), right_operand(j, i),
                               preferred_element_type=jnp.float32)
            return m

        ln = {}
        lhs = {}
        done = {}
        for waits, norm, prods in _STARTUP:
            for name in waits:
                wait(name)
            for blk in norm:
                ln[blk] = [ln_piece(blk, q) for q in range(_NQ)]
            for blk, _ in prods:
                if blk not in lhs:
                    lhs[blk] = left_operands(ln[blk])
            tied = [blk for blk in norm if prods and blk not in [p[0] for p in prods]]
            nslots = 7 * len(prods)
            if not tied and len(prods) == 2 and prods[0][1] == prods[1][1]:
                j = prods[0][1]
                stacked = [jnp.concatenate([lhs[blk][i] for blk, _ in prods], axis=0)
                           for i in range(7)]
                m = products(stacked, j, lambda s: [])
                for bi, (blk, _) in enumerate(prods):
                    combine(blk, j, {i: m[i][bi * _R:(bi + 1) * _R] for i in range(7)})
                    done[blk] = done.get(blk, 0) + 1
                continue
            for pi, (blk, j) in enumerate(prods):
                def masks_for_slot(s, pi=pi):
                    slot = pi * 7 + s
                    return [ln[tb][q][1] for tb in tied for q in range(_NQ - 1)
                            if min(nslots - 1, 6 + (q * (nslots - 6)) // (_NQ - 1)) == slot]
                combine(blk, j, products(lhs[blk], j, masks_for_slot))
                done[blk] = done.get(blk, 0) + 1
                if done[blk] == 4:
                    out_start(blk, 0, N)

        cur = ln[_N_STARTUP]
        for blk in range(_N_STARTUP, nb):
            a_ops = left_operands(cur)
            nxt = None
            if blk + 1 < nb:
                wait("x%d" % blk_group[blk + 1])
                if blk_group[blk + 1] == len(_X_GROUPS) - 1 and not released[0]:
                    release_outputs()
                nxt = [ln_piece(blk + 1, q) for q in range(_NQ)]
            for j in range(4):
                def masks_for_slot(s, j=j):
                    if nxt is None:
                        return []
                    return [nxt[q][1] for q in range(_NQ - 1) if _TIE_SLOTS[q] == j * 7 + s]
                combine(blk, j, products(a_ops, j, masks_for_slot))
                if blk == nb - 1:
                    out_start(blk, j * 128, (j + 1) * 128)
                    out_start(blk, H + j * 128, H + (j + 1) * 128)
            if blk != nb - 1:
                out_start(blk, 0, N)
            cur = nxt

        for cp in out_copies:
            cp.wait()

    return kernel


@jax.jit
def pallas_standalone__layernorm_linear__prompt_kernel(
    x: jax.Array,
    g: jax.Array,
    b: jax.Array,
    w: jax.Array,
):
    B, S, D = x.shape
    M, N = B * S, w.shape[1]
    nb = M // _BR
    hbm = pl.BlockSpec(memory_space=pl.ANY)
    out = pl.pallas_call(
        _make_kernel(M, D, N),
        in_specs=[hbm] * 4,
        out_specs=hbm,
        out_shape=jax.ShapeDtypeStruct((M, N), x.dtype),
        scratch_shapes=[
            pltpu.VMEM((M, D), x.dtype),
            pltpu.VMEM((8, 128), g.dtype),
            pltpu.VMEM((8, 128), b.dtype),
            pltpu.VMEM((D, N), w.dtype),
            pltpu.SemaphoreType.DMA((len(_X_GROUPS),)),
            pltpu.SemaphoreType.DMA((2,)),
            pltpu.SemaphoreType.DMA((8,)),
            pltpu.SemaphoreType.DMA(()),
            pltpu.SemaphoreType.REGULAR(()),
        ] + [pltpu.VMEM((_BR, N), x.dtype) for _ in range(nb)],
        compiler_params=pltpu.CompilerParams(
            vmem_limit_bytes=100 * 1024 * 1024,
            disable_semaphore_checks=True,
            flags={"XLA_TPU_EVENLY_DISTRIBUTE_CRITICAL_NODES": True},
        ),
    )(x.reshape(M, D), g.reshape(8, 128), b.reshape(8, 128), w)
    return out.reshape(B, S, N)
```
